```python
import os as _os
_os.environ.setdefault("JAX_PLATFORMS", "cpu")
import jax
import jax.numpy as jnp

def _softmax(x, axis=-1):
    return jax.nn.softmax(x, axis=axis)
def _gelu(x):
    return jax.nn.gelu(x, approximate=True)
def _silu(x):
    return jax.nn.silu(x)
def _sigmoid(x):
    return jax.nn.sigmoid(x)
def _layernorm(x, axis=-1, eps=1e-5):
    m = jnp.mean(x, axis=axis, keepdims=True)
    v = jnp.var(x, axis=axis, keepdims=True)
    return (x - m) / jnp.sqrt(v + eps)
def _scatter_add(tgt, idx, src, axis=0):
    return tgt.at[idx].add(src)
def _segment_sum(src, seg, n):
    return jax.ops.segment_sum(src, seg, n)
class _Rng:
    def __init__(self, key):
        self._k = key
    def _next(self):
        self._k, sub = jax.random.split(self._k)
        return sub
    def normal(self, shape):
        return jax.random.normal(self._next(), shape, dtype=jnp.bfloat16)
    def randint(self, lo, hi, shape):
        return jax.random.randint(self._next(), shape, lo, hi, dtype=jnp.int32)
    def uniform(self, shape, lo=0.0, hi=1.0):
        return jax.random.uniform(self._next(), shape, jnp.bfloat16, lo, hi)
    def permutation(self, n):
        return jax.random.permutation(self._next(), n)


kernel_name = 'gated_mix__ssm_conv_s5__geglu_ffn__prompt'

def setup_inputs():
    _rng = _Rng(jax.random.key(int.from_bytes(__import__("os").urandom(4), "little")))
    _w = (lambda a: (lambda t: t.astype(jnp.bfloat16) if jnp.issubdtype(t.dtype, jnp.floating) else t)(jnp.asarray(a)))
    def _A_setup():
        B, S, D = 1, 2048, 512
        P = D
        Lambda_re = -0.5 * jnp.exp((lambda *s: _rng.normal(s) * 0.4)(P))
        Lambda_im = (lambda *s: _rng.normal(s) * 0.4)(P) * 1.0
        B_re = (lambda *s: _rng.normal(s) * 0.4)(P, D) * (D ** -0.5)
        B_im = (lambda *s: _rng.normal(s) * 0.4)(P, D) * (D ** -0.5)
        C_re = (lambda *s: _rng.normal(s) * 0.4)(D, P) * (P ** -0.5)
        C_im = (lambda *s: _rng.normal(s) * 0.4)(D, P) * (P ** -0.5)
        log_dt = (lambda *s: _rng.normal(s) * 0.4)(P) * 0.3 - 2.0
        Dskip = (lambda *s: _rng.normal(s) * 0.4)(D)
        return {
            "x": _w((lambda *s: _rng.normal(s) * 0.05)(B, S, D)),
            "Lambda_re": _w(Lambda_re),
            "Lambda_im": _w(Lambda_im),
            "B_re": _w(B_re),
            "B_im": _w(B_im),
            "C_re": _w(C_re),
            "C_im": _w(C_im),
            "log_dt": _w(log_dt),
            "Dskip": _w(Dskip),
        }
    _A_in = _A_setup()

    def _B_setup():
        B, S, D, F = 1, 2048, 512, 1376
        return {
            "x": _w((lambda *s: _rng.normal(s) * 0.05)(B, S, D)),
            "w_gate": _w((lambda *s: _rng.normal(s) * 0.1)(D, F)),
            "w_up": _w((lambda *s: _rng.normal(s) * 0.1)(D, F)),
            "w_down": _w((lambda *s: _rng.normal(s) * 0.1)(F, D)),
        }
    _B_in = _B_setup()

    return {
        "A_x": _A_in["x"],
        "A_Lambda_re": _A_in["Lambda_re"],
        "A_Lambda_im": _A_in["Lambda_im"],
        "A_B_re": _A_in["B_re"],
        "A_B_im": _A_in["B_im"],
        "A_C_re": _A_in["C_re"],
        "A_C_im": _A_in["C_im"],
        "A_log_dt": _A_in["log_dt"],
        "A_Dskip": _A_in["Dskip"],
        "B_x": _B_in["x"],
        "B_w_gate": _B_in["w_gate"],
        "B_w_up": _B_in["w_up"],
        "B_w_down": _B_in["w_down"],
        "gate_w": _w((lambda *s: _rng.normal(s) * 0.05)(512) * 16.0),
    }

def reference(A_x, A_Lambda_re, A_Lambda_im, A_B_re, A_B_im, A_C_re, A_C_im, A_log_dt, A_Dskip, B_x, B_w_gate, B_w_up, B_w_down, gate_w):
    def _A_ref(x, Lambda_re, Lambda_im, B_re, B_im, C_re, C_im, log_dt, Dskip):
        Bsz, L, H = x.shape
        Lam = Lambda_re + 1j * Lambda_im
        Bmat = B_re + 1j * B_im
        Cmat = C_re + 1j * C_im
        dt = jnp.exp(log_dt)
        Lam_bar = jnp.exp(dt * Lam)
        B_bar = ((Lam_bar - 1.0) / Lam)[:, None] * Bmat
        Bu = jnp.einsum("bld,pd->blp", x + 0j, B_bar)
        h = jnp.zeros_like(Bu[:, 0, :])
        hs = []
        for t in range(L):
            h = Lam_bar[None, :] * h + Bu[:, t, :]
            hs.append(h)
        hseq = jnp.stack(hs, 1)
        y = 2.0 * jnp.einsum("blp,dp->bld", hseq, Cmat).real + x * Dskip[None, None, :]
        return y

    def _B_ref(x, w_gate, w_up, w_down):
        return (_gelu(x @ w_gate) * (x @ w_up)) @ w_down

    x = A_x
    g = _sigmoid((x * gate_w).sum(-1, keepdims=True))
    a = _A_ref(x, A_Lambda_re, A_Lambda_im, A_B_re, A_B_im, A_C_re, A_C_im, A_log_dt, A_Dskip)
    b = _B_ref(x, B_w_gate, B_w_up, B_w_down)
    return g * a + (1 - g) * b
```

```python
import jax
import jax.numpy as jnp
import jax.experimental.pallas as pl
import jax.experimental.pallas.tpu as pltpu

T_CHUNK = 256
_NT = (((1,), (1,)), ((), ()))


def _nt(a, b):
    return jax.lax.dot_general(a, b, _NT, preferred_element_type=jnp.float32)


def _cmul(ar, ai, br, bi):
    return ar * br - ai * bi, ar * bi + ai * br


def _kernel(x_ref, lre_ref, lim_ref, ldt_ref, dsk_ref, gw_ref,
            bre_hbm, bim_hbm, cre_hbm, cim_hbm, wgt_hbm, wut_hbm, wd_hbm,
            o_ref,
            bst_s, cst_s, wgt_s, wut_s, wd_s,
            bbar_s, cc_s, coef_s, h_s, carry_s, sems):
    T, D = x_ref.shape
    P = lre_ref.shape[-1]
    f32 = jnp.float32
    bf16 = jnp.bfloat16

    def copies():
        return [
            pltpu.make_async_copy(bre_hbm, bst_s.at[0], sems.at[0]),
            pltpu.make_async_copy(bim_hbm, bst_s.at[1], sems.at[1]),
            pltpu.make_async_copy(wgt_hbm, wgt_s, sems.at[2]),
            pltpu.make_async_copy(wut_hbm, wut_s, sems.at[3]),
            pltpu.make_async_copy(wd_hbm, wd_s, sems.at[4]),
            pltpu.make_async_copy(cre_hbm, cst_s.at[0], sems.at[5]),
            pltpu.make_async_copy(cim_hbm, cst_s.at[1], sems.at[6]),
        ]

    def row(ref):
        return ref[...].astype(f32).reshape(1, -1)

    def body(first):
        if first:
            cps = copies()
            for cp in cps:
                cp.start()
            lre = row(lre_ref)
            lim = row(lim_ref)
            dt = jnp.exp(row(ldt_ref)).astype(bf16).astype(f32)
            ar = dt * lre
            ai = dt * lim
            mag = jnp.exp(ar)
            lbr = mag * jnp.cos(ai)
            lbi = mag * jnp.sin(ai)
            nr = lbr - 1.0
            ni = lbi
            den = lre * lre + lim * lim
            cr = (nr * lre + ni * lim) / den
            ci = (ni * lre - nr * lim) / den
            pw = [(lbr, lbi)]
            for _ in range(7):
                pw.append(_cmul(pw[-1][0], pw[-1][1], lbr, lbi))
            rid = jax.lax.broadcasted_iota(jnp.int32, (8, P), 0)
            zero = jnp.zeros((8, P), f32)
            for n, k in enumerate((1, 2, 4)):
                coef_s[2 * n] = jnp.where(rid >= k, jnp.broadcast_to(pw[k - 1][0], (8, P)), zero)
                coef_s[2 * n + 1] = jnp.where(rid >= k, jnp.broadcast_to(pw[k - 1][1], (8, P)), zero)
            pr = zero
            pi = zero
            for j in range(8):
                pr = jnp.where(rid == j, jnp.broadcast_to(pw[j][0], (8, P)), pr)
                pi = jnp.where(rid == j, jnp.broadcast_to(pw[j][1], (8, P)), pi)
            coef_s[6] = pr
            coef_s[7] = pi
            carry_s[...] = jnp.zeros_like(carry_s)
            crc = jnp.broadcast_to(cr, (128, P)).T
            cic = jnp.broadcast_to(ci, (128, P)).T
            cps[0].wait()
            cps[1].wait()
            for j in range(D // 128):
                sl = slice(j * 128, (j + 1) * 128)
                br = bst_s[0, :, sl].astype(f32)
                bi = bst_s[1, :, sl].astype(f32)
                bbar_s[:P, sl] = (crc * br - cic * bi).astype(bf16)
                bbar_s[P:, sl] = (cic * br + crc * bi).astype(bf16)

        xb = x_ref[...]
        bu = _nt(xb, bbar_s[...])

        c_r = carry_s[0:1, :P]
        c_i = carry_s[0:1, P:]
        for g2 in range(T // 16):
            halves = []
            for hh in range(2):
                r0 = g2 * 16 + hh * 8
                vr = bu[r0:r0 + 8, :P]
                vi = bu[r0:r0 + 8, P:]
                for n, k in enumerate((1, 2, 4)):
                    sr = pltpu.roll(vr, k, 0)
                    si = pltpu.roll(vi, k, 0)
                    mr, mi = _cmul(coef_s[2 * n], coef_s[2 * n + 1], sr, si)
                    vr = vr + mr
                    vi = vi + mi
                mr, mi = _cmul(coef_s[6], coef_s[7],
                               jnp.broadcast_to(c_r, (8, P)), jnp.broadcast_to(c_i, (8, P)))
                vr = vr + mr
                vi = vi + mi
                c_r = vr[7:8, :]
                c_i = vi[7:8, :]
                halves.append((vr, vi))
            hr = jnp.concatenate([halves[0][0], halves[1][0]], axis=0).astype(bf16)
            hi = jnp.concatenate([halves[0][1], halves[1][1]], axis=0).astype(bf16)
            h_s[g2 * 16:(g2 + 1) * 16, :P] = hr
            h_s[g2 * 16:(g2 + 1) * 16, P:] = hi
        carry_s[0:1, :P] = c_r
        carry_s[0:1, P:] = c_i

        if first:
            cps[2].wait()
        gate = _nt(xb, wgt_s[...])
        if first:
            cps[3].wait()
        up = _nt(xb, wut_s[...])
        hid = (jax.nn.gelu(gate, approximate=True) * up).astype(bf16)
        if first:
            cps[4].wait()
        ffn = jnp.dot(hid, wd_s[...], preferred_element_type=f32)

        if first:
            cps[5].wait()
            cps[6].wait()
            cc_s[:, :P] = (2.0 * cst_s[0].astype(f32)).astype(bf16)
            cc_s[:, P:] = (-2.0 * cst_s[1].astype(f32)).astype(bf16)
        y = _nt(h_s[...], cc_s[...])

        xf = xb.astype(f32)
        g = jax.nn.sigmoid(jnp.sum(xf * row(gw_ref), axis=-1, keepdims=True))
        a = y + xf * row(dsk_ref)
        o_ref[...] = g * a + (1.0 - g) * ffn

    @pl.when(pl.program_id(0) == 0)
    def _():
        body(True)

    @pl.when(pl.program_id(0) != 0)
    def _():
        body(False)


@jax.jit
def pallas_gated_mix__ssm_conv_s5__geglu_ffn__prompt_kernel(
    A_x, A_Lambda_re, A_Lambda_im, A_B_re, A_B_im, A_C_re, A_C_im, A_log_dt,
    A_Dskip, B_x, B_w_gate, B_w_up, B_w_down, gate_w,
):
    Bsz, L, D = A_x.shape
    P = A_Lambda_re.shape[0]
    F = B_w_gate.shape[1]
    assert Bsz == 1 and L % T_CHUNK == 0
    x2 = A_x.reshape(L, D)
    vec = lambda n: pl.BlockSpec((n,), lambda i: (0,))
    hbm = pl.BlockSpec(memory_space=pl.ANY)
    bf16 = jnp.bfloat16
    out = pl.pallas_call(
        _kernel,
        grid=(L // T_CHUNK,),
        in_specs=[
            pl.BlockSpec((T_CHUNK, D), lambda i: (i, 0)),
            vec(P), vec(P), vec(P), vec(D), vec(D),
            hbm, hbm, hbm, hbm, hbm, hbm, hbm,
        ],
        out_specs=pl.BlockSpec((T_CHUNK, D), lambda i: (i, 0)),
        out_shape=jax.ShapeDtypeStruct((L, D), jnp.float32),
        scratch_shapes=[
            pltpu.VMEM((2, P, D), bf16),
            pltpu.VMEM((2, D, P), bf16),
            pltpu.VMEM((F, D), bf16),
            pltpu.VMEM((F, D), bf16),
            pltpu.VMEM((F, D), bf16),
            pltpu.VMEM((2 * P, D), bf16),
            pltpu.VMEM((D, 2 * P), bf16),
            pltpu.VMEM((8, 8, P), jnp.float32),
            pltpu.VMEM((T_CHUNK, 2 * P), bf16),
            pltpu.VMEM((8, 2 * P), jnp.float32),
            pltpu.SemaphoreType.DMA((7,)),
        ],
        compiler_params=pltpu.CompilerParams(
            dimension_semantics=("arbitrary",),
            vmem_limit_bytes=64 * 1024 * 1024,
        ),
    )(x2, A_Lambda_re, A_Lambda_im, A_log_dt, A_Dskip, gate_w,
      A_B_re, A_B_im, A_C_re, A_C_im, B_w_gate.T, B_w_up.T, B_w_down)
    return out.reshape(Bsz, L, D)
```

```python
import jax
import jax.numpy as jnp
import jax.experimental.pallas as pl
import jax.experimental.pallas.tpu as pltpu

T_CHUNK = 256
K_AHEAD = 1
_NT = (((1,), (1,)), ((), ()))


def _nt(a, b):
    return jax.lax.dot_general(a, b, _NT, preferred_element_type=jnp.float32)


def _cmul(ar, ai, br, bi):
    return ar * br - ai * bi, ar * bi + ai * br


def _kernel(x_ref, x_hbm, lre_ref, lim_ref, ldt_ref, dsk_ref, gw_ref,
            bre_hbm, bim_hbm, cre_hbm, cim_hbm, wgt_hbm, wut_hbm, wd_hbm,
            o_ref,
            xa_s, ua_s, b_s, cst_s, wgt_s, wut_s, wd_s,
            cc_s, coef_s, h_s, carry_s, sems):
    T, D = o_ref.shape
    P = lre_ref.shape[-1]
    KA = xa_s.shape[0]
    f32 = jnp.float32
    bf16 = jnp.bfloat16
    step = pl.program_id(0)

    def row(ref):
        return ref[...].astype(f32).reshape(1, -1)

    def body(mode):
        first = mode == "first"
        if first:
            cps = [
                pltpu.make_async_copy(bre_hbm, b_s.at[pl.ds(0, P), :], sems.at[0]),
                pltpu.make_async_copy(bim_hbm, b_s.at[pl.ds(P, P), :], sems.at[1]),
                pltpu.make_async_copy(wgt_hbm, wgt_s, sems.at[2]),
                pltpu.make_async_copy(wut_hbm, wut_s, sems.at[3]),
                pltpu.make_async_copy(wd_hbm, wd_s, sems.at[4]),
                pltpu.make_async_copy(cre_hbm, cst_s.at[0], sems.at[5]),
                pltpu.make_async_copy(cim_hbm, cst_s.at[1], sems.at[6]),
            ]
            xcp = [pltpu.make_async_copy(x_hbm.at[pl.ds((k + 1) * T, T), :], xa_s.at[k], sems.at[7 + k])
                   for k in range(KA)]
            cps[0].start()
            cps[1].start()
            for cp in xcp:
                cp.start()
            for cp in cps[2:]:
                cp.start()

            lre = row(lre_ref)
            lim = row(lim_ref)
            dt = jnp.exp(row(ldt_ref)).astype(bf16).astype(f32)
            ar = dt * lre
            ai = dt * lim
            mag = jnp.exp(ar)
            lbr = mag * jnp.cos(ai)
            lbi = mag * jnp.sin(ai)
            nr = lbr - 1.0
            ni = lbi
            den = lre * lre + lim * lim
            cr = (nr * lre + ni * lim) / den
            ci = (ni * lre - nr * lim) / den
            pw = [(lbr, lbi)]
            for _ in range(3):
                pw.append(_cmul(pw[-1][0], pw[-1][1], lbr, lbi))
            rid = jax.lax.broadcasted_iota(jnp.int32, (8, P), 0)
            zero = jnp.zeros((8, P), f32)
            for n, k in enumerate((1, 2, 4)):
                coef_s[2 * n] = jnp.where(rid >= k, jnp.broadcast_to(pw[k - 1][0], (8, P)), zero)
                coef_s[2 * n + 1] = jnp.where(rid >= k, jnp.broadcast_to(pw[k - 1][1], (8, P)), zero)
            coef_s[6] = jnp.where(rid == 0, jnp.broadcast_to(lbr, (8, P)), zero)
            coef_s[7] = jnp.where(rid == 0, jnp.broadcast_to(lbi, (8, P)), zero)
            carry_s[...] = jnp.zeros_like(carry_s)

        xb = x_ref[...]
        if first:
            cps[0].wait()
            u_r = _nt(xb, b_s[:P, :])
            cps[1].wait()
            u_i = _nt(xb, b_s[P:, :])
        elif mode == "pre":
            u_r = ua_s[step - 1, :, :P]
            u_i = ua_s[step - 1, :, P:]
        else:
            u = _nt(xb, b_s[...])
            u_r = u[:, :P]
            u_i = u[:, P:]

        c_r = carry_s[0:1, :P]
        c_i = carry_s[0:1, P:]
        for g2 in range(T // 16):
            halves = []
            for hh in range(2):
                r0 = g2 * 16 + hh * 8
                vr = u_r[r0:r0 + 8, :]
                vi = u_i[r0:r0 + 8, :]
                mr, mi = _cmul(coef_s[6], coef_s[7],
                               jnp.broadcast_to(c_r, (8, P)), jnp.broadcast_to(c_i, (8, P)))
                vr = vr + mr
                vi = vi + mi
                for n, k in enumerate((1, 2, 4)):
                    sr = pltpu.roll(vr, k, 0)
                    si = pltpu.roll(vi, k, 0)
                    mr, mi = _cmul(coef_s[2 * n], coef_s[2 * n + 1], sr, si)
                    vr = vr + mr
                    vi = vi + mi
                c_r = vr[7:8, :]
                c_i = vi[7:8, :]
                halves.append((vr, vi))
            hr = jnp.concatenate([halves[0][0], halves[1][0]], axis=0).astype(bf16)
            hi = jnp.concatenate([halves[0][1], halves[1][1]], axis=0).astype(bf16)
            h_s[g2 * 16:(g2 + 1) * 16, :P] = hr
            h_s[g2 * 16:(g2 + 1) * 16, P:] = hi
        carry_s[0:1, :P] = c_r
        carry_s[0:1, P:] = c_i

        if first:
            for k in range(KA):
                xcp[k].wait()
                ua_s[k] = _nt(xa_s[k], b_s[...])
            cps[2].wait()
        gate = _nt(xb, wgt_s[...])
        if first:
            cps[3].wait()
        up = _nt(xb, wut_s[...])
        hid = (jax.nn.gelu(gate, approximate=True) * up).astype(bf16)
        if first:
            cps[4].wait()
        ffn = jnp.dot(hid, wd_s[...], preferred_element_type=f32)

        if first:
            cps[5].wait()
            cps[6].wait()
            c_re = cst_s[0].astype(f32)
            c_im = cst_s[1].astype(f32)
            cc_s[:, :P] = (2.0 * (c_re * cr - c_im * ci)).astype(bf16)
            cc_s[:, P:] = (-2.0 * (c_re * ci + c_im * cr)).astype(bf16)
        y = _nt(h_s[...], cc_s[...])

        xf = xb.astype(f32)
        g = jax.nn.sigmoid(jnp.sum(xf * row(gw_ref), axis=-1, keepdims=True))
        a = y + xf * row(dsk_ref)
        o_ref[...] = g * a + (1.0 - g) * ffn

    @pl.when(step == 0)
    def _():
        body("first")

    @pl.when(jnp.logical_and(step >= 1, step <= KA))
    def _():
        body("pre")

    @pl.when(step > KA)
    def _():
        body("normal")


@jax.jit
def pallas_gated_mix__ssm_conv_s5__geglu_ffn__prompt_kernel(
    A_x, A_Lambda_re, A_Lambda_im, A_B_re, A_B_im, A_C_re, A_C_im, A_log_dt,
    A_Dskip, B_x, B_w_gate, B_w_up, B_w_down, gate_w,
):
    Bsz, L, D = A_x.shape
    P = A_Lambda_re.shape[0]
    F = B_w_gate.shape[1]
    assert Bsz == 1 and L % T_CHUNK == 0 and L // T_CHUNK > K_AHEAD
    x2 = A_x.reshape(L, D)
    hbm = pl.BlockSpec(memory_space=pl.ANY)
    vec = lambda n: pl.BlockSpec((n,), lambda i: (0,))
    bf16 = jnp.bfloat16
    out = pl.pallas_call(
        _kernel,
        grid=(L // T_CHUNK,),
        in_specs=[pl.BlockSpec((T_CHUNK, D), lambda i: (i, 0)), hbm,
                  vec(P), vec(P), vec(P), vec(D), vec(D)] + [hbm] * 7,
        out_specs=pl.BlockSpec((T_CHUNK, D), lambda i: (i, 0)),
        out_shape=jax.ShapeDtypeStruct((L, D), jnp.float32),
        scratch_shapes=[
            pltpu.VMEM((K_AHEAD, T_CHUNK, D), bf16),
            pltpu.VMEM((K_AHEAD, T_CHUNK, 2 * P), jnp.float32),
            pltpu.VMEM((2 * P, D), bf16),
            pltpu.VMEM((2, D, P), bf16),
            pltpu.VMEM((F, D), bf16),
            pltpu.VMEM((F, D), bf16),
            pltpu.VMEM((F, D), bf16),
            pltpu.VMEM((D, 2 * P), bf16),
            pltpu.VMEM((8, 8, P), jnp.float32),
            pltpu.VMEM((T_CHUNK, 2 * P), bf16),
            pltpu.VMEM((8, 2 * P), jnp.float32),
            pltpu.SemaphoreType.DMA((7 + K_AHEAD,)),
        ],
        compiler_params=pltpu.CompilerParams(
            dimension_semantics=("arbitrary",),
            vmem_limit_bytes=64 * 1024 * 1024,
        ),
    )(x2, x2, A_Lambda_re, A_Lambda_im, A_log_dt, A_Dskip, gate_w,
      A_B_re, A_B_im, A_C_re, A_C_im, B_w_gate.T, B_w_up.T, B_w_down)
    return out.reshape(Bsz, L, D)
```
